```python
import jax
import jax.numpy as jnp

def _softmax(x, axis=-1):
    return jax.nn.softmax(x, axis=axis)
def _gelu(x):
    return jax.nn.gelu(x, approximate=True)
def _silu(x):
    return jax.nn.silu(x)
def _sigmoid(x):
    return jax.nn.sigmoid(x)
def _layernorm(x, axis=-1, eps=1e-5):
    m = jnp.mean(x, axis=axis, keepdims=True)
    v = jnp.var(x, axis=axis, keepdims=True)
    return (x - m) / jnp.sqrt(v + eps)
def _scatter_add(tgt, idx, src, axis=0):
    return tgt.at[idx].add(src)
def _segment_sum(src, seg, n):
    return jax.ops.segment_sum(src, seg, n)
class _Rng:
    def __init__(self, key):
        self._k = key
    def _next(self):
        self._k, sub = jax.random.split(self._k)
        return sub
    def normal(self, shape):
        return jax.random.normal(self._next(), shape, dtype=jnp.bfloat16)
    def randint(self, lo, hi, shape):
        return jax.random.randint(self._next(), shape, lo, hi, dtype=jnp.int32)
    def uniform(self, shape, lo=0.0, hi=1.0):
        return jax.random.uniform(self._next(), shape, jnp.bfloat16, lo, hi)
    def permutation(self, n):
        return jax.random.permutation(self._next(), n)


kernel_name = 'standalone__structured_sparse_n_m__ragged'

def setup_inputs():
    _rng = _Rng(jax.random.key(int.from_bytes(__import__("os").urandom(4), "little")))
    _w = (lambda a: (lambda t: t.astype(jnp.bfloat16) if jnp.issubdtype(t.dtype, jnp.floating) else t)(jnp.asarray(a)))
    B, S, D = 16, 4096, 576
    assert D % 4 == 0, "d_model must be divisible by M=4 for 2:4 sparsity"
    return {
        "x": _w((lambda *s: _rng.normal(s) * 0.05)(B, S, D)),
        "w": _w((lambda *s: _rng.normal(s) * 0.05)(D, D)),
        "b": _w((lambda *s: _rng.normal(s) * 0.05)(D)),
    }

def reference(x, w, b):
    B, S, D = x.shape
    N, M = 2, 4
    G = D // M
    wg = w.reshape(G, M, D)
    mag = jnp.abs(wg)
    order = jnp.argsort(mag, 1)
    thr = jnp.take_along_axis(mag, order[:, M - N:M - N + 1, :], 1)
    mask = (lambda x, dt: x.astype(dt))(mag >= thr, w.dtype)
    wp = (wg * mask).reshape(D, D)
    return jnp.einsum("bsd,df->bsf", x, wp) + b
```

```python
import functools
import jax, jax.numpy as jnp
import jax.experimental.pallas as pl
import jax.experimental.pallas.tpu as pltpu

def make(TS=1024, vmem=64*1024*1024):
    def kern(x_ref, w_ref, b_ref, o_ref, wt_ref):
        @pl.when((pl.program_id(0)==0) & (pl.program_id(1)==0))
        def _():
            w = w_ref[...].astype(jnp.float32)
            mag = jnp.abs(w)
            row = jax.lax.broadcasted_iota(jnp.int32, w.shape, 0)
            odd = (row & 1) == 1
            hi = (row & 2) == 2
            D = w.shape[0]
            p1 = jnp.where(odd, pltpu.roll(mag, 1, 0), pltpu.roll(mag, D-1, 0))
            mx = jnp.maximum(mag, p1); mn = jnp.minimum(mag, p1)
            mx2 = jnp.where(hi, pltpu.roll(mx, 2, 0), pltpu.roll(mx, D-2, 0))
            mn2 = jnp.where(hi, pltpu.roll(mn, 2, 0), pltpu.roll(mn, D-2, 0))
            thr = jnp.maximum(jnp.minimum(mx, mx2), jnp.maximum(mn, mn2))
            wp = jnp.where(mag >= thr, w, 0.0)
            wt_ref[...] = wp.T.astype(jnp.bfloat16)
        acc = jnp.dot(wt_ref[...], x_ref[...], preferred_element_type=jnp.float32)
        o_ref[...] = (acc + b_ref[...].astype(jnp.float32)).astype(o_ref.dtype)

    def fn(x, w, b):
        B,S,D = x.shape
        xt = jnp.swapaxes(x,1,2)
        out = pl.pallas_call(
            kern,
            grid=(B, S//TS),
            in_specs=[pl.BlockSpec((None, D, TS), lambda i,j:(i,0,j)),
                      pl.BlockSpec((D,D), lambda i,j:(0,0)),
                      pl.BlockSpec((D,1), lambda i,j:(0,0))],
            out_specs=pl.BlockSpec((None, D, TS), lambda i,j:(i,0,j)),
            out_shape=jax.ShapeDtypeStruct((B,D,S), x.dtype),
            scratch_shapes=[pltpu.VMEM((D,D), jnp.bfloat16)],
            compiler_params=pltpu.CompilerParams(dimension_semantics=("arbitrary","arbitrary"), vmem_limit_bytes=vmem),
        )(xt, w, b.reshape(D,1))
        return jnp.swapaxes(out,1,2)
    return fn

@jax.jit
def pallas_standalone__structured_sparse_n_m__ragged_kernel(x, w, b):
    return make(2048)(x, w, b)
```

```python
import functools
import jax, jax.numpy as jnp
import numpy as np
import jax.experimental.pallas as pl
import jax.experimental.pallas.tpu as pltpu
from jax import lax

D = 576
KP = 640
SL = 4096

F = jnp.float32; I = jnp.int32
def mask_vreg(u, idx):
    lo = pltpu.bitcast((u << 16) & 0x7FFFFFFF, F)
    hi = pltpu.bitcast(u & 0x7FFF0000, F)
    mx = jnp.maximum(lo, hi); mn = jnp.minimum(lo, hi)
    mx2 = jnp.take_along_axis(mx, idx, axis=0); mn2 = jnp.take_along_axis(mn, idx, axis=0)
    thr = jnp.maximum(jnp.minimum(mx, mx2), jnp.maximum(mn, mn2))
    keep = jnp.where(lo < thr, 0, 0xFFFF) | jnp.where(hi < thr, 0, -65536)
    return u & keep

def prep4(w_ref, b_ref, wt_ref):
    idx = lax.broadcasted_iota(jnp.int32, (8,128), 0) ^ 1
    cols = []
    for c in range(0, D, 128):
        rows = []
        for r in range(0, D, 16):
            if c + 128 <= D:
                v = w_ref[r:r+16, c:c+128]
            else:
                v = w_ref[r:r+16, c:D]
                v = jnp.concatenate([v, jnp.zeros((16, c+128-D), v.dtype)], axis=1)
            u = pltpu.bitcast(v, I)
            rows.append(pltpu.bitcast(mask_vreg(u, idx), jnp.bfloat16))
        cols.append(jnp.concatenate(rows, axis=0))
    wp = jnp.concatenate(cols, axis=1)
    b = b_ref[...].astype(jnp.float32).reshape(1, D)
    b = jnp.concatenate([b, jnp.zeros((1, KP-D), F)], axis=1)
    r0 = lax.broadcasted_iota(jnp.int32, (16, KP), 0) == 0
    ex = [jnp.where(r0, jnp.broadcast_to(b, (16, KP)), 0.0).astype(jnp.bfloat16), jnp.zeros((KP-D-16, KP), jnp.bfloat16)]
    wa = jnp.concatenate([wp] + ex, axis=0)
    wt_ref[...] = wa[:, :D].T

def make(up=(512,1024,2560), G=6144, PC=2048, OUTC=512, pad=0, NOB=2, vmem=124*1024*1024, nochk=True, last=(256,256), dbg=0):
    U = sum(up); assert U == SL
    NC = 16*SL
    m = (NC - U)//G; assert m*G + U == NC
    assert G % PC == 0 and SL % PC == 0
    nup = len(up)
    cum = np.concatenate([[0], np.cumsum(up)]).tolist()

    def kern(x_hbm, w_hbm, b_hbm, o_hbm, w_ref, b_ref, wt_ref, xb, o0, ob, sin, sout):
        def mm(xv, n):
            cst = (lax.broadcasted_iota(jnp.int32, (KP-D, n), 0) == 0).astype(jnp.bfloat16)
            xa = jnp.concatenate([xv, cst], axis=0)
            return jnp.dot(wt_ref[...], xa, preferred_element_type=jnp.float32).astype(jnp.bfloat16)
        def in_piece(s, c0, n, sem):
            return pltpu.make_async_copy(x_hbm.at[s, :, pl.ds(c0, n)], xb.at[s, :, pl.ds(c0, n)], sem)
        def group_in(g):
            cps = []
            c = U + g*G; e = c + G
            while c < e:
                n = min(e, (c//SL+1)*SL) - c
                cps.append(in_piece(c//SL, c % SL, n, sin.at[nup + g]))
                c += n
            return cps
        semw = sin.at[nup+m]
        wc = pltpu.make_async_copy(w_hbm, w_ref, semw); wc.start()
        bc = pltpu.make_async_copy(b_hbm, b_ref, semw); bc.start()
        for i in range(nup): in_piece(0, cum[i], up[i], sin.at[i]).start()
        for g in range(m):
            for cp in group_in(g): cp.start()
        wc.wait(); bc.wait()
        if not (dbg & 4): prep4(w_ref, b_ref, wt_ref)
        for i in range(nup):
            if not (dbg & 2): in_piece(0, cum[i], up[i], sin.at[i]).wait()
            o0[:, cum[i]:cum[i+1]] = mm(xb[0, :, cum[i]:cum[i+1]], up[i])
        def grp_wait(sem):
            pltpu.make_async_copy(ob.at[0], xg_dst, sem).wait()
        def step(g, carry):
            slot = (g & 1) if NOB == 2 else g % NOB
            if not (dbg & 1): pltpu.make_async_copy(x_hbm.at[pl.ds(0, G//PC), :, pl.ds(0, PC)], ob.at[0], sin.at[nup + g]).wait()
            @pl.when(g == 0)
            def _():
                pltpu.make_async_copy(o0, o_hbm.at[0], sout.at[NOB]).start()
            @pl.when(g >= NOB)
            def _():
                pltpu.make_async_copy(ob.at[0], o_hbm.at[pl.ds(0, G//PC), :, pl.ds(0, PC)], sout.at[slot]).wait()
            c = U + g*G
            for p in range(G//PC):
                cp = c + p*PC
                s = lax.shift_right_logical(cp, 12)
                c0 = pl.multiple_of(cp & (SL-1), PC)
                sizes = [OUTC]*(PC//OUTC)
                if p == G//PC - 1 and last: sizes = sizes[:-1] + list(last)
                o = 0
                for n in sizes:
                    ob[slot, p, :, o:o+n] = mm(xb[s, :, pl.ds(pl.multiple_of(c0 + o, 128), n)], n)
                    pltpu.make_async_copy(ob.at[slot, p, :, pl.ds(o, n)], o_hbm.at[s, :, pl.ds(pl.multiple_of(c0 + o, 128), n)], sout.at[slot]).start()
                    o += n
            return carry
        lax.fori_loop(0, m, step, 0)
        if dbg & 1:
            for g in range(m): pltpu.make_async_copy(x_hbm.at[pl.ds(0, G//PC), :, pl.ds(0, PC)], ob.at[0], sin.at[nup + g]).wait()
        if dbg & 2:
            for i in range(nup): in_piece(0, cum[i], up[i], sin.at[i]).wait()
        pltpu.make_async_copy(o0, o_hbm.at[0], sout.at[NOB]).wait()
        for sl in range(NOB):
            pltpu.make_async_copy(ob.at[0], o_hbm.at[pl.ds(0, G//PC), :, pl.ds(0, PC)], sout.at[sl]).wait()

    def fn(x, w, b):
        B,S,_ = x.shape
        xt = jnp.swapaxes(x,1,2)
        out = pl.pallas_call(
            kern,
            in_specs=[pl.BlockSpec(memory_space=pl.ANY)]*3,
            out_specs=pl.BlockSpec(memory_space=pl.ANY),
            out_shape=jax.ShapeDtypeStruct((B,D,S), x.dtype),
            scratch_shapes=[pltpu.VMEM((D,D), jnp.bfloat16), pltpu.VMEM((D,), jnp.bfloat16), pltpu.VMEM((D,KP), jnp.bfloat16),
                            pltpu.VMEM((B,D,SL+pad), jnp.bfloat16), pltpu.VMEM((D,SL), jnp.bfloat16), pltpu.VMEM((NOB,G//PC,D,PC), jnp.bfloat16),
                            pltpu.SemaphoreType.DMA((nup+m+1,)), pltpu.SemaphoreType.DMA((NOB+1,))],
            compiler_params=pltpu.CompilerParams(vmem_limit_bytes=vmem, disable_bounds_checks=nochk),
        )(xt, w, b)
        return jnp.swapaxes(out,1,2)
    return fn


@jax.jit
def pallas_standalone__structured_sparse_n_m__ragged_kernel(x, w, b):
    return make(G=6144, pad=128, OUTC=2048, last=(1024, 512, 256, 128, 128))(x, w, b)
```
